```python
import os as _os
_os.environ.setdefault("JAX_PLATFORMS", "cpu")
import jax
import jax.numpy as jnp

def _softmax(x, axis=-1):
    return jax.nn.softmax(x, axis=axis)
def _gelu(x):
    return jax.nn.gelu(x, approximate=True)
def _silu(x):
    return jax.nn.silu(x)
def _sigmoid(x):
    return jax.nn.sigmoid(x)
def _layernorm(x, axis=-1, eps=1e-5):
    m = jnp.mean(x, axis=axis, keepdims=True)
    v = jnp.var(x, axis=axis, keepdims=True)
    return (x - m) / jnp.sqrt(v + eps)
def _scatter_add(tgt, idx, src, axis=0):
    return tgt.at[idx].add(src)
def _segment_sum(src, seg, n):
    return jax.ops.segment_sum(src, seg, n)
class _Rng:
    def __init__(self, key):
        self._k = key
    def _next(self):
        self._k, sub = jax.random.split(self._k)
        return sub
    def normal(self, shape):
        return jax.random.normal(self._next(), shape, dtype=jnp.bfloat16)
    def randint(self, lo, hi, shape):
        return jax.random.randint(self._next(), shape, lo, hi, dtype=jnp.int32)
    def uniform(self, shape, lo=0.0, hi=1.0):
        return jax.random.uniform(self._next(), shape, jnp.bfloat16, lo, hi)
    def permutation(self, n):
        return jax.random.permutation(self._next(), n)


kernel_name = 'gated_mix__ssm_conv_s5__geglu_ffn__prompt'

def setup_inputs():
    _rng = _Rng(jax.random.key(int.from_bytes(__import__("os").urandom(4), "little")))
    _w = (lambda a: (lambda t: t.astype(jnp.bfloat16) if jnp.issubdtype(t.dtype, jnp.floating) else t)(jnp.asarray(a)))
    def _A_setup():
        B, S, D = 1, 2048, 512
        P = D
        Lambda_re = -0.5 * jnp.exp((lambda *s: _rng.normal(s) * 0.4)(P))
        Lambda_im = (lambda *s: _rng.normal(s) * 0.4)(P) * 1.0
        B_re = (lambda *s: _rng.normal(s) * 0.4)(P, D) * (D ** -0.5)
        B_im = (lambda *s: _rng.normal(s) * 0.4)(P, D) * (D ** -0.5)
        C_re = (lambda *s: _rng.normal(s) * 0.4)(D, P) * (P ** -0.5)
        C_im = (lambda *s: _rng.normal(s) * 0.4)(D, P) * (P ** -0.5)
        log_dt = (lambda *s: _rng.normal(s) * 0.4)(P) * 0.3 - 2.0
        Dskip = (lambda *s: _rng.normal(s) * 0.4)(D)
        return {
            "x": _w((lambda *s: _rng.normal(s) * 0.05)(B, S, D)),
            "Lambda_re": _w(Lambda_re),
            "Lambda_im": _w(Lambda_im),
            "B_re": _w(B_re),
            "B_im": _w(B_im),
            "C_re": _w(C_re),
            "C_im": _w(C_im),
            "log_dt": _w(log_dt),
            "Dskip": _w(Dskip),
        }
    _A_in = _A_setup()

    def _B_setup():
        B, S, D, F = 1, 2048, 512, 1376
        return {
            "x": _w((lambda *s: _rng.normal(s) * 0.05)(B, S, D)),
            "w_gate": _w((lambda *s: _rng.normal(s) * 0.1)(D, F)),
            "w_up": _w((lambda *s: _rng.normal(s) * 0.1)(D, F)),
            "w_down": _w((lambda *s: _rng.normal(s) * 0.1)(F, D)),
        }
    _B_in = _B_setup()

    return {
        "A_x": _A_in["x"],
        "A_Lambda_re": _A_in["Lambda_re"],
        "A_Lambda_im": _A_in["Lambda_im"],
        "A_B_re": _A_in["B_re"],
        "A_B_im": _A_in["B_im"],
        "A_C_re": _A_in["C_re"],
        "A_C_im": _A_in["C_im"],
        "A_log_dt": _A_in["log_dt"],
        "A_Dskip": _A_in["Dskip"],
        "B_x": _B_in["x"],
        "B_w_gate": _B_in["w_gate"],
        "B_w_up": _B_in["w_up"],
        "B_w_down": _B_in["w_down"],
        "gate_w": _w((lambda *s: _rng.normal(s) * 0.05)(512) * 16.0),
    }

def reference(A_x, A_Lambda_re, A_Lambda_im, A_B_re, A_B_im, A_C_re, A_C_im, A_log_dt, A_Dskip, B_x, B_w_gate, B_w_up, B_w_down, gate_w):
    def _A_ref(x, Lambda_re, Lambda_im, B_re, B_im, C_re, C_im, log_dt, Dskip):
        Bsz, L, H = x.shape
        Lam = Lambda_re + 1j * Lambda_im
        Bmat = B_re + 1j * B_im
        Cmat = C_re + 1j * C_im
        dt = jnp.exp(log_dt)
        Lam_bar = jnp.exp(dt * Lam)
        B_bar = ((Lam_bar - 1.0) / Lam)[:, None] * Bmat
        Bu = jnp.einsum("bld,pd->blp", x + 0j, B_bar)
        h = jnp.zeros_like(Bu[:, 0, :])
        hs = []
        for t in range(L):
            h = Lam_bar[None, :] * h + Bu[:, t, :]
            hs.append(h)
        hseq = jnp.stack(hs, 1)
        y = 2.0 * jnp.einsum("blp,dp->bld", hseq, Cmat).real + x * Dskip[None, None, :]
        return y

    def _B_ref(x, w_gate, w_up, w_down):
        return (_gelu(x @ w_gate) * (x @ w_up)) @ w_down

    x = A_x
    g = _sigmoid((x * gate_w).sum(-1, keepdims=True))
    a = _A_ref(x, A_Lambda_re, A_Lambda_im, A_B_re, A_B_im, A_C_re, A_C_im, A_log_dt, A_Dskip)
    b = _B_ref(x, B_w_gate, B_w_up, B_w_down)
    return g * a + (1 - g) * b
```

```python
import jax
import jax.numpy as jnp
from jax import lax
import jax.experimental.pallas as pl
import jax.experimental.pallas.tpu as pltpu

L, D, P, F = 2048, 512, 512, 1376
NS = 8
SEG = L // NS
TJ = 32
NB = SEG // TJ
TB = NS * TJ
TJP = TJ + 8
NC = D // 128
FC = 256
PR = 32
WR = 32
WSTAGE = 5
PRI_X = 0
PRI_W = 1
GR = 32
MR = 64
F32 = jnp.float32
BF16 = jnp.bfloat16
NT = (((1,), (1,)), ((), ()))


def _cmul(ar, ai, br, bi):
    return ar * br - ai * bi, ar * bi + ai * br


def _gelu(g):
    inner = 0.7978845608028654 * (g + 0.044715 * (g * g * g))
    return 0.5 * g * (1.0 + jnp.tanh(inner))


def _run(*timed):
    items = [it for lst in timed for it in lst]
    for n in sorted(range(len(items)), key=lambda k: (items[k][0], k)):
        items[n][1]()


def _seq(t0, pieces):
    out = []
    for dur, fn in pieces:
        out.append((t0, fn))
        t0 += dur
    return out, t0


def _spread(t0, t1, fns):
    fns = list(fns)
    return [(t0 + (t1 - t0) * (n + 0.25) / len(fns), fn) for n, fn in enumerate(fns)]


def _kernel(x_hbm, lre_hbm, lim_hbm, bre_hbm, bim_hbm, cre_hbm, cim_hbm, ldt_hbm, dsk_hbm,
            wg_hbm, wu_hbm, wd_hbm, gw_hbm, out_hbm,
            lre_v, lim_v, ldt_v, dsk_v, gw_v,
            x_v, xf_v, xp0_v, xp1_v, b_v, c_v, cw_v, wg_v, wu_v, wd_v, bu_v, h0_v, h1_v, acc_v, g_v, y_v, st_v, xs_v, t_v, gu_v, a0_v, a1_v,
            xsem, osem, wsem, vsem, bsem):
    cols = [pl.ds(128 * c, 128) for c in range(NC)]

    st5_v = st_v.reshape(NB, NC, NS, TJP, 128)

    def x_copy(i, n=1):
        return pltpu.make_async_copy(x_hbm.at[:, pl.ds(i, n)], x_v.at[:, pl.ds(i, n)], xsem.at[i])

    def whole(buf, sem):
        return pltpu.make_async_copy(buf, buf, sem)

    def o_copy(i, c):
        return pltpu.make_async_copy(st5_v.at[i, c, :, pl.ds(0, TJ), :],
                                     out_hbm.at[:, i, :, cols[c]], osem.at[i])

    def w_copies(k, src, dst, r0, n):
        return [pltpu.make_async_copy(src.at[:, cols[c]], dst.at[c, pl.ds(r0, n)], wsem.at[k])
                for c in range(NC)]

    QB = 2 * P // 4
    cb = [[pltpu.make_async_copy((bre_hbm, bim_hbm)[q // 2].at[pl.ds(QB * (q % 2), QB), cols[c]],
                                 b_v.at[c, pl.ds(QB * q, QB)], bsem.at[q]) for c in range(NC)]
          for q in range(4)]
    wait_b = lambda q: whole(b_v.at[:, pl.ds(QB * q, QB)], bsem.at[q]).wait()
    cc_re = w_copies(2, cre_hbm, c_v, 0, D)
    cc_im = w_copies(3, cim_hbm, c_v, D, D)
    c_wg = w_copies(4, wg_hbm, wg_v, 0, F)
    c_wu = w_copies(5, wu_hbm, wu_v, 0, F)
    c_wd = w_copies(6, wd_hbm, wd_v, 0, F)
    vec_copies = [pltpu.make_async_copy(s, d, vsem.at[k]) for k, (s, d) in enumerate(
        ((lre_hbm, lre_v), (lim_hbm, lim_v), (ldt_hbm, ldt_v), (dsk_hbm, dsk_v), (gw_hbm, gw_v)))]

    def start(cs):
        for c in cs:
            c.start()

    def wait(cs):
        for c in cs:
            c.wait()

    x_copy(0).start()
    start(cb[0])
    start(vec_copies)
    U32 = jnp.uint32
    bw_v, cin_v = b_v.bitcast(U32), c_v.bitcast(U32)
    cww_v = cw_v.bitcast(U32)
    xp_l, h_l, a_l = (xp0_v, xp1_v), (h0_v, h1_v), (a0_v, a1_v)
    xpw_l, hw_l, aw_l = ([r.bitcast(U32) for r in l] for l in (xp_l, h_l, a_l))
    xsw_v, tw_v = xs_v.bitcast(U32), t_v.bitcast(U32)
    wgw_v, wuw_v, wdw_v = wg_v.bitcast(U32), wu_v.bitcast(U32), wd_v.bitcast(U32)

    def ld(ref, idx, r0, n):
        return pltpu.bitcast(ref[(*idx, pl.ds(r0 // 2, n // 2), slice(None))], BF16)

    def stb(ref, idx, r0, val):
        ref[(*idx, pl.ds(r0, val.shape[0]), slice(None))] = val

    def lanes(ref, idx, nc, r0, n):
        return jnp.concatenate([ld(ref, (*idx, c), r0, n) for c in range(nc)], axis=1)

    def perm_a(i, c, s):
        def fn():
            xf_v[c, pl.ds(TJP * s, TJ), :] = x_v[s, i, :, cols[c]].astype(F32)
        return fn

    def perm_as(i):
        return [perm_a(i, c, s) for c in (0, 2, 1, 3) for s in range(NS)]

    HB = TB // 2

    def perm_b(i, c, r0):
        def fn():
            rows = lambda cc, r: jnp.concatenate(
                [xf_v[cc, pl.ds(j, NS, stride=TJP), :] for j in range(r // NS, (r + PR) // NS)], axis=0)
            a11, a21, a12, a22 = rows(c, r0), rows(c, HB + r0), rows(c + 2, r0), rows(c + 2, HB + r0)
            stb(xp_l[i % 2], (i // 2, c), r0, a11.astype(BF16))
            stb(xp_l[i % 2], (i // 2, c), HB + r0, a21.astype(BF16))
            stb(xp_l[i % 2], (i // 2, c + 2), r0, a12.astype(BF16))
            stb(xp_l[i % 2], (i // 2, c + 2), HB + r0, a22.astype(BF16))
            for k, v in enumerate((a11 + a22, a21 + a22, a11 + a12, a21 - a11, a12 - a22)):
                stb(xs_v, (i, k, c), r0, v.astype(BF16))
        return fn

    def perm_bs(i):
        return [perm_b(i, c, r0) for c in range(2) for r0 in range(0, HB, PR)]

    def wprep(c, r0, n):
        def fn():
            b11 = ld(wgw_v, (c,), r0, n).astype(F32)
            b21 = ld(wgw_v, (c + 2,), r0, n).astype(F32)
            b12 = ld(wuw_v, (c,), r0, n).astype(F32)
            b22 = ld(wuw_v, (c + 2,), r0, n).astype(F32)
            for k, v in enumerate((b11 + b22, b12 - b22, b21 - b11, b11 + b12, b21 + b22)):
                stb(t_v, (k, c), r0, v.astype(BF16))
        return fn

    def bu_mm(i, n):
        def fn():
            w = lanes(bw_v, (), NC, 128 * n, 128)
            bu_v[i, n] = lax.dot_general(lanes(xpw_l[i % 2], (i // 2,), NC, 0, TB), w, NT, preferred_element_type=F32)
        return fn

    st = {}

    def scan(i, j, store):
        def fn():
            er, ei = st["er"], st["ei"]
            lr, li = st["lr"], st["li"]
            for c in range(NC):
                hs = []
                for jj in (j, j + 1):
                    br = bu_v[i, c, pl.ds(NS * jj, NS), :]
                    bi = bu_v[i, NC + c, pl.ds(NS * jj, NS), :]
                    er[c], ei[c] = lr[c] * er[c] - li[c] * ei[c] + br, lr[c] * ei[c] + li[c] * er[c] + bi
                    hs.append((er[c], ei[c]))
                if store:
                    stb(h_l[i % 2], (c,), NS * j, jnp.concatenate([hs[0][0], hs[1][0]], axis=0).astype(BF16))
                    stb(h_l[i % 2], (NC + c,), NS * j, jnp.concatenate([hs[0][1], hs[1][1]], axis=0).astype(BF16))
        return fn

    def scans(i, store):
        return [scan(i, j, store) for j in range(0, TJ, 2)]

    def ffn_items(i, t0):
        val = {}
        two = lambda ref, idx, k0, r0, m: jnp.concatenate([ld(ref, (*idx, k0 + c), r0, m) for c in range(2)], axis=1)
        lhs = ((xsw_v, (i, 0), 0, 0), (xsw_v, (i, 1), 0, 0), (xpw_l[i % 2], (i // 2,), 0, 0), (xpw_l[i % 2], (i // 2,), 2, HB),
               (xsw_v, (i, 2), 0, 0), (xsw_v, (i, 3), 0, 0), (xsw_v, (i, 4), 0, 0))
        rhs = ((tw_v, (0,), 0), (wgw_v, (), 0), (tw_v, (1,), 0), (tw_v, (2,), 0),
               (wuw_v, (), 2), (tw_v, (3,), 0), (tw_v, (4,), 0))

        def prod(q, k, c0, n):
            def fn():
                ref, idx, k0, r0 = lhs[k]
                m = lax.dot_general(two(ref, idx, k0, r0, HB), two(*rhs[k], c0, n), NT, preferred_element_type=F32)
                if k == 0:
                    val["g1"], val["u2"] = m, m
                elif k == 1:
                    val["g2"], val["u2"] = m, val["u2"] - m
                elif k == 2:
                    val["u1"], val["u2"] = m, val["u2"] + m
                elif k == 3:
                    val["g1"] = val["g1"] + m
                    gu_v[q % 2, 2, :, 0:n] = val.pop("g2") + m
                elif k == 4:
                    val["g1"] = val["g1"] - m
                    gu_v[q % 2, 1, :, 0:n] = val.pop("u1") + m
                elif k == 5:
                    gu_v[q % 2, 3, :, 0:n] = val.pop("u2") + m
                else:
                    gu_v[q % 2, 0, :, 0:n] = val.pop("g1") + m
            return fn

        def act(q, h, c, n):
            def fn():
                w = min(128, n - 128 * c)
                cs = pl.ds(128 * c, w)
                a = (_gelu(gu_v[q % 2, 2 * h, :, cs]) * gu_v[q % 2, 2 * h + 1, :, cs]).astype(BF16)
                a_l[q % 2][c, pl.ds(HB * h, HB), 0:w] = a
            return fn

        def down(q, c0, n):
            def fn():
                if n == FC:
                    a = jnp.concatenate([ld(aw_l[q % 2], (c,), 0, TB) for c in range(FC // 128)], axis=1)
                else:
                    a = a_l[q % 2][0, :, 0:n]
                d = jnp.dot(a, lanes(wdw_v, (), NC, c0, n), preferred_element_type=F32)
                if q == 0:
                    acc_v[i % 2] = d
                else:
                    acc_v[i % 2] += d
            return fn

        items, t, marks = [], t0, []
        pend = None
        for q, (c0, c1) in enumerate(chunks):
            n = c1 - c0
            nt = (n + 127) // 128
            for k in range(7):
                items.append((t, prod(q, k, c0, n)))
                if k == 0:
                    marks.append(t)
                t += nt * T
            tq = t
            parts = [act(q, h, c, n) for c in range(nt) for h in range(2)]
            if pend is not None:
                items.append((t, pend))
                t += 8 * T
            items += [(tq + T + 4 * T * j, f) for j, f in enumerate(parts)]
            pend = down(q, c0, n)
        return items, t, pend, marks

    def gate(i, r0, nr):
        def fn():
            z = None
            for c in range(NC):
                t = (xp_l[i % 2][i // 2, c, pl.ds(r0, nr), :].astype(F32) * st["gw"][c]).astype(BF16).astype(F32)
                z = t if z is None else z + t
            z = jnp.sum(z, axis=-1, keepdims=True).astype(BF16).astype(F32)
            g_v[i % 2, pl.ds(r0, nr), :] = jnp.broadcast_to(jax.nn.sigmoid(z), (nr, 128))
        return fn

    def gates(i):
        return [gate(i, r0, GR) for r0 in range(0, TB, GR)]

    def cproj(i, n):
        def fn():
            y_v[n] = lax.dot_general(lanes(hw_l[i % 2], (), 2 * NC, 0, TB),
                                     lanes(cww_v, (), 2 * NC, 128 * n, 128), NT, preferred_element_type=F32)
        return fn

    def mix(i, n, r0, nr):
        def fn():
            xf = ld(xpw_l[i % 2], (i // 2, n), r0, nr).astype(F32)
            g = g_v[i % 2, pl.ds(r0, nr), :]
            a = y_v[n, pl.ds(r0, nr), :] + (xf * st["dsk"][n]).astype(BF16).astype(F32)
            res = g * a + (1.0 - g) * acc_v[i % 2, pl.ds(r0, nr), cols[n]]
            for j in range(r0 // NS, (r0 + nr) // NS):
                st_v[i, n, pl.ds(j, NS, stride=TJP), :] = res[NS * j - r0:NS * j - r0 + NS, :]
            if r0 + nr == TB and i >= NB - 1:
                o_copy(i, n).start()
        return fn

    def mixes(i, n):
        return [mix(i, n, r0, MR) for r0 in range(0, TB, MR)]

    def discretise():
        wait(vec_copies)
        lre = lre_v[...].astype(F32).reshape(1, P)
        lim = lim_v[...].astype(F32).reshape(1, P)
        dt = jnp.exp(ldt_v[...].astype(F32).reshape(1, P)).astype(BF16).astype(F32)
        mag = jnp.exp(dt * lre)
        lr1 = mag * jnp.cos(dt * lim)
        li1 = mag * jnp.sin(dt * lim)
        den = lre * lre + lim * lim
        nr = lr1 - 1.0
        st["kr"] = (nr * lre + li1 * lim) / den
        st["ki"] = (li1 * lre - nr * lim) / den
        lr = jnp.broadcast_to(lr1, (NS, P))
        li = jnp.broadcast_to(li1, (NS, P))
        tiles = lambda v: [v[:, 128 * c:128 * (c + 1)] for c in range(NC)]
        st["lr"], st["li"] = tiles(lr), tiles(li)
        pr, pi = lr1, li1
        for _ in range(8):
            pr, pi = _cmul(pr, pi, pr, pi)
        st["pr"], st["pi"] = tiles(jnp.broadcast_to(pr, (NS, P))), tiles(jnp.broadcast_to(pi, (NS, P)))
        z = jnp.zeros((NS, 128), F32)
        st["er"], st["ei"] = [z] * NC, [z] * NC
        st["gw"] = tiles(gw_v[...].astype(F32).reshape(1, D))
        st["dsk"] = tiles(dsk_v[...].astype(F32).reshape(1, D))

    def cprep(c, h):
        def fn():
            cr = ld(cin_v, (c,), 128 * h, 128).astype(F32)
            ci = ld(cin_v, (c,), D + 128 * h, 128).astype(F32)
            kr, ki = st["kr"][:, 128 * c:128 * (c + 1)], st["ki"][:, 128 * c:128 * (c + 1)]
            wr, wi = _cmul(cr, ci, kr, ki)
            stb(cw_v, (c,), 128 * h, (2.0 * wr).astype(BF16))
            stb(cw_v, (NC + c,), 128 * h, (-2.0 * wi).astype(BF16))
        return fn

    def carry():
        sub = lax.broadcasted_iota(jnp.int32, (NS, 128), 0)
        for c in range(NC):
            ar, ai = st["pr"][c], st["pi"][c]
            er, ei = st["er"][c], st["ei"][c]
            for k in (1, 2, 4):
                sr = jnp.where(sub >= k, pltpu.roll(er, k, 0), 0.0)
                si = jnp.where(sub >= k, pltpu.roll(ei, k, 0), 0.0)
                tr, ti = _cmul(ar, ai, sr, si)
                er, ei = er + tr, ei + ti
                ar, ai = _cmul(ar, ai, ar, ai)
            st["er"][c] = jnp.where(sub >= 1, pltpu.roll(er, 1, 0), 0.0)
            st["ei"][c] = jnp.where(sub >= 1, pltpu.roll(ei, 1, 0), 0.0)

    x_copy(0).wait()
    start(cb[1])
    for f in perm_as(0) + perm_bs(0):
        f()
    discretise()
    wait_b(0)
    start(cb[2] + [x_copy(1)])
    starts = {1: [x_copy(4, 4)], 2: c_wg, 3: c_wu, WSTAGE: c_wd + cc_re + cc_im}
    waits = {1: [x_copy(2, 2)], 3: [x_copy(4, 4)], WSTAGE: [whole(wg_v, wsem.at[4]), whole(wu_v, wsem.at[5])]}
    wp = [wprep(c, r0, min(WR, F - r0)) for r0 in range(0, F, WR) for c in range(2)]
    T = 16 * TB // 64

    for i in range(NB):
        main = [(4 * T, bu_mm(i, n)) for n in range(2 * NC)]
        if i == 0:
            main[6:6] = [(0, lambda: (wait_b(3), x_copy(1).wait()))]
            main[4:4] = [(0, lambda: (wait_b(2), x_copy(2, 2).start()))]
            main[2:2] = [(0, lambda: (wait_b(1), start(cb[3])))]
        main, t1 = _seq(0, main)
        side = []
        wait(waits.get(i, []))
        start(starts.get(i, []))
        if i == 0:
            side += _spread(t1 * 0.75 + 1, t1 * 0.87, perm_as(1)) + _spread(t1 * 0.87, t1, perm_bs(1))
        elif i + 1 < NB:
            side += _spread(0, t1 * 0.5, perm_as(i + 1))
            side += _spread(t1 * 0.5, t1, perm_bs(i + 1))
        if i >= 1:
            side += _spread(0, t1, scans(i - 1, False))
        side += _spread(0, t1, wp[len(wp) * (i - WSTAGE) // (NB - WSTAGE):len(wp) * (i + 1 - WSTAGE) // (NB - WSTAGE)] if i >= WSTAGE else [])
        _run(main, side)

    chunks = [(c0, min(c0 + FC, F)) for c0 in range(0, F, FC)]
    pend_down = None
    for i in range(NB + 1):
        main, side, t1 = [], [], 0
        if i < NB:
            first, t1, last, marks = ffn_items(i, 0)
            main += first
        if i >= 1:
            tp = 14 * T if i < NB else 0
            shift = 4 * T + 8 * T * NC
            main = [(t + (shift if t >= tp else 0), f) for t, f in main]
            main.append((tp, pend_down))
            main += [(tp + 4 * T + 8 * T * n, cproj(i - 1, n)) for n in range(NC)]
            t1 += shift
            tm = tp + shift
        if i == NB:
            side += [(tp + 4 * T + 8 * T * (n + 1) - 1, f) for n in range(NC) for f in mixes(i - 1, n)]
        elif i >= 1:
            side += _spread(tm + 4 * T, tm + 60 * T, [f for n in range(NC) for f in mixes(i - 1, n)])
            td = min(t + shift for t in marks if t + shift > tm + 60 * T)
            side += [(td + 0.5, lambda i=i: start([o_copy(i - 1, c) for c in range(NC)]))]
            side += _spread(tm + 60 * T, t1, gates(i))
            side += _spread(0, t1 - 8 * T, scans(i, True))
        else:
            side += _spread(70 * T, t1, gates(0))
            side += _spread(0, 30 * T, scans(NB - 1, False))
            side += [(30 * T, carry), (marks[1] + 0.5, lambda: wait([whole(wd_v, wsem.at[6]), whole(c_v.at[:, pl.ds(0, D)], wsem.at[2]),
                                                         whole(c_v.at[:, pl.ds(D, D)], wsem.at[3])]))]
            side += _spread(30 * T, 70 * T, [cprep(c, h) for c in range(NC) for h in range(D // 128)])
            side += _spread(40 * T, t1 - 8 * T, scans(i, True))
        if i < NB:
            pend_down = last
        _run(main, side)
    for i in range(NB):
        pltpu.make_async_copy(st5_v.at[i, :, :, pl.ds(0, TJ), :], st5_v.at[i, :, :, pl.ds(0, TJ), :], osem.at[i]).wait()


@jax.jit
def pallas_gated_mix__ssm_conv_s5__geglu_ffn__prompt_kernel(
    A_x, A_Lambda_re, A_Lambda_im, A_B_re, A_B_im, A_C_re, A_C_im, A_log_dt, A_Dskip,
    B_x, B_w_gate, B_w_up, B_w_down, gate_w,
):
    del B_x
    x4 = A_x.reshape(NS, NB, TJ, D)
    hbm = pl.BlockSpec(memory_space=pltpu.HBM)
    out = pl.pallas_call(
        _kernel,
        out_shape=jax.ShapeDtypeStruct((NS, NB, TJ, D), F32),
        in_specs=[hbm] * 13,
        out_specs=hbm,
        scratch_shapes=[
            *[pltpu.VMEM((P,), BF16)] * 5,
            pltpu.VMEM((NS, NB, TJ, D), BF16),
            pltpu.VMEM((NC, NS * TJP, 128), F32),
            *[pltpu.VMEM((NB // 2, NC, TB, 128), BF16)] * 2,
            pltpu.VMEM((NC, 2 * P, 128), BF16),
            pltpu.VMEM((NC, 2 * D, 128), BF16),
            pltpu.VMEM((2 * NC, D, 128), BF16),
            pltpu.VMEM((NC, F, 128), BF16),
            pltpu.VMEM((NC, F, 128), BF16),
            pltpu.VMEM((NC, F, 128), BF16),
            pltpu.VMEM((NB, 2 * NC, TB, 128), F32),
            *[pltpu.VMEM((2 * NC, TB, 128), BF16)] * 2,
            pltpu.VMEM((2, TB, D), F32),
            pltpu.VMEM((2, TB, 128), F32),
            pltpu.VMEM((NC, TB, 128), F32),
            pltpu.VMEM((NB, NC, NS * TJP, 128), F32),
            pltpu.VMEM((NB, 5, 2, TB // 2, 128), BF16),
            pltpu.VMEM((5, 2, F, 128), BF16),
            pltpu.VMEM((2, 4, TB // 2, FC), F32),
            *[pltpu.VMEM((FC // 128, TB, 128), BF16)] * 2,
            pltpu.SemaphoreType.DMA((NB,)),
            pltpu.SemaphoreType.DMA((NB,)),
            pltpu.SemaphoreType.DMA((7,)),
            pltpu.SemaphoreType.DMA((5,)),
            pltpu.SemaphoreType.DMA((4,)),
        ],
        compiler_params=pltpu.CompilerParams(vmem_limit_bytes=64 * 1024 * 1024),
    )(x4, A_Lambda_re, A_Lambda_im, A_B_re, A_B_im, A_C_re, A_C_im, A_log_dt, A_Dskip,
      B_w_gate.T, B_w_up.T, B_w_down, gate_w)
    return out.reshape(1, L, D)
```

```python
import jax
import jax.numpy as jnp
from jax import lax
import jax.experimental.pallas as pl
import jax.experimental.pallas.tpu as pltpu

L, D, P, F = 2048, 512, 512, 1376
NS = 8
SEG = L // NS
TJ = 32
NB = SEG // TJ
TB = NS * TJ
TJP = TJ + 8
NC = D // 128
FC = 256
PR = 32
WR = 32
WSTAGE = 5
CPQ = 2
MIXT = 40
XSTAGE = 2
GR = 32
MR = 64
F32 = jnp.float32
BF16 = jnp.bfloat16
NT = (((1,), (1,)), ((), ()))


def _cmul(ar, ai, br, bi):
    return ar * br - ai * bi, ar * bi + ai * br


def _gelu(g):
    inner = 0.7978845608028654 * (g + 0.044715 * (g * g * g))
    return 0.5 * g * (1.0 + jnp.tanh(inner))


def _run(*timed):
    items = [it for lst in timed for it in lst]
    for n in sorted(range(len(items)), key=lambda k: (items[k][0], k)):
        items[n][1]()


def _seq(t0, pieces):
    out = []
    for dur, fn in pieces:
        out.append((t0, fn))
        t0 += dur
    return out, t0


def _spread(t0, t1, fns):
    fns = list(fns)
    return [(t0 + (t1 - t0) * (n + 0.25) / len(fns), fn) for n, fn in enumerate(fns)]


def _kernel(x_hbm, lre_hbm, lim_hbm, bre_hbm, bim_hbm, cre_hbm, cim_hbm, ldt_hbm, dsk_hbm,
            wg_hbm, wu_hbm, wd_hbm, gw_hbm, out_hbm,
            lre_v, lim_v, ldt_v, dsk_v, gw_v,
            x_v, xf_v, xp0_v, xp1_v, b_v, c_v, cw_v, wg_v, wu_v, wd_v, bu_v, h0_v, h1_v, acc_v, g_v, y_v, st_v, xs0_v, xs1_v, t_v, gu_v, a0_v, a1_v,
            xsem, osem, wsem, vsem, bsem):
    cols = [pl.ds(128 * c, 128) for c in range(NC)]

    st5_v = st_v.reshape(NB, NC, NS, TJP, 128)

    def x_copy(i, n=1):
        return pltpu.make_async_copy(x_hbm.at[:, pl.ds(i, n)], x_v.at[:, pl.ds(i, n)], xsem.at[i])

    def whole(buf, sem):
        return pltpu.make_async_copy(buf, buf, sem)

    def o_copy(i, c):
        return pltpu.make_async_copy(st5_v.at[i, c, :, pl.ds(0, TJ), :],
                                     out_hbm.at[:, i, :, cols[c]], osem.at[i])

    def w_copies(k, src, dst, r0, n):
        return [pltpu.make_async_copy(src.at[:, cols[c]], dst.at[c, pl.ds(r0, n)], wsem.at[k])
                for c in range(NC)]

    QB = 2 * P // 4
    cb = [[pltpu.make_async_copy((bre_hbm, bim_hbm)[q // 2].at[pl.ds(QB * (q % 2), QB), cols[c]],
                                 b_v.at[c, pl.ds(QB * q, QB)], bsem.at[q]) for c in range(NC)]
          for q in range(4)]
    wait_b = lambda q: whole(b_v.at[:, pl.ds(QB * q, QB)], bsem.at[q]).wait()
    cc_re = w_copies(2, cre_hbm, c_v, 0, D)
    cc_im = w_copies(3, cim_hbm, c_v, D, D)
    c_wg = w_copies(4, wg_hbm, wg_v, 0, F)
    c_wu = w_copies(5, wu_hbm, wu_v, 0, F)
    c_wd = w_copies(6, wd_hbm, wd_v, 0, F)
    vec_copies = [pltpu.make_async_copy(s, d, vsem.at[k]) for k, (s, d) in enumerate(
        ((lre_hbm, lre_v), (lim_hbm, lim_v), (ldt_hbm, ldt_v), (dsk_hbm, dsk_v), (gw_hbm, gw_v)))]

    def start(cs):
        for c in cs:
            c.start()

    def wait(cs):
        for c in cs:
            c.wait()

    x_copy(0).start()
    start(cb[0])
    start(vec_copies)
    U32 = jnp.uint32
    bw_v, cin_v = b_v.bitcast(U32), c_v.bitcast(U32)
    cww_v = cw_v.bitcast(U32)
    xp_l, h_l, a_l = (xp0_v, xp1_v), (h0_v, h1_v), (a0_v, a1_v)
    xpw_l, hw_l, aw_l = ([r.bitcast(U32) for r in l] for l in (xp_l, h_l, a_l))
    xs_l = (xs0_v, xs1_v)
    xsw_l, tw_v = [r.bitcast(U32) for r in xs_l], t_v.bitcast(U32)
    wgw_v, wuw_v, wdw_v = wg_v.bitcast(U32), wu_v.bitcast(U32), wd_v.bitcast(U32)

    def ld(ref, idx, r0, n):
        return pltpu.bitcast(ref[(*idx, pl.ds(r0 // 2, n // 2), slice(None))], BF16)

    def stb(ref, idx, r0, val):
        ref[(*idx, pl.ds(r0, val.shape[0]), slice(None))] = val

    def lanes(ref, idx, nc, r0, n):
        return jnp.concatenate([ld(ref, (*idx, c), r0, n) for c in range(nc)], axis=1)

    def perm_a(i, c, s):
        def fn():
            xf_v[c, pl.ds(TJP * s, TJ), :] = x_v[s, i, :, cols[c]].astype(F32)
        return fn

    def perm_as(i):
        return [perm_a(i, c, s) for c in (0, 2, 1, 3) for s in range(NS)]

    HB = TB // 2

    def perm_b(i, c, r0):
        def fn():
            rows = lambda cc, r: jnp.concatenate(
                [xf_v[cc, pl.ds(j, NS, stride=TJP), :] for j in range(r // NS, (r + PR) // NS)], axis=0)
            a11, a21, a12, a22 = rows(c, r0), rows(c, HB + r0), rows(c + 2, r0), rows(c + 2, HB + r0)
            stb(xp_l[i % 2], (i // 2, c), r0, a11.astype(BF16))
            stb(xp_l[i % 2], (i // 2, c), HB + r0, a21.astype(BF16))
            stb(xp_l[i % 2], (i // 2, c + 2), r0, a12.astype(BF16))
            stb(xp_l[i % 2], (i // 2, c + 2), HB + r0, a22.astype(BF16))
        return fn

    def xsum(i, c, r0):
        def fn():
            q = lambda cc, r: ld(xpw_l[i % 2], (i // 2, cc), r, PR).astype(F32)
            a11, a21, a12, a22 = q(c, r0), q(c, HB + r0), q(c + 2, r0), q(c + 2, HB + r0)
            for k, v in enumerate((a11 + a22, a21 + a22, a11 + a12, a21 - a11, a12 - a22)):
                stb(xs_l[i % 2], (k, c), r0, v.astype(BF16))
        return fn

    def xsums(i):
        return [xsum(i, c, r0) for c in range(2) for r0 in range(0, HB, PR)]

    def perm_bs(i):
        return [perm_b(i, c, r0) for c in range(2) for r0 in range(0, HB, PR)]

    def wprep(c, r0, n):
        def fn():
            b11 = ld(wgw_v, (c,), r0, n).astype(F32)
            b21 = ld(wgw_v, (c + 2,), r0, n).astype(F32)
            b12 = ld(wuw_v, (c,), r0, n).astype(F32)
            b22 = ld(wuw_v, (c + 2,), r0, n).astype(F32)
            for k, v in enumerate((b11 + b22, b12 - b22, b21 - b11, b11 + b12, b21 + b22)):
                stb(t_v, (k, c), r0, v.astype(BF16))
        return fn

    def bu_mm(i, n):
        def fn():
            w = lanes(bw_v, (), NC, 128 * n, 128)
            bu_v[i, n] = lax.dot_general(lanes(xpw_l[i % 2], (i // 2,), NC, 0, TB), w, NT, preferred_element_type=F32)
        return fn

    st = {}

    def scan(i, j, store):
        def fn():
            er, ei = st["er"], st["ei"]
            lr, li = st["lr"], st["li"]
            for c in range(NC):
                hs = []
                for jj in (j, j + 1):
                    br = bu_v[i, c, pl.ds(NS * jj, NS), :]
                    bi = bu_v[i, NC + c, pl.ds(NS * jj, NS), :]
                    er[c], ei[c] = lr[c] * er[c] - li[c] * ei[c] + br, lr[c] * ei[c] + li[c] * er[c] + bi
                    hs.append((er[c], ei[c]))
                if store:
                    stb(h_l[i % 2], (c,), NS * j, jnp.concatenate([hs[0][0], hs[1][0]], axis=0).astype(BF16))
                    stb(h_l[i % 2], (NC + c,), NS * j, jnp.concatenate([hs[0][1], hs[1][1]], axis=0).astype(BF16))
        return fn

    def scans(i, store):
        return [scan(i, j, store) for j in range(0, TJ, 2)]

    def ffn_items(i, t0):
        val = {}
        two = lambda ref, idx, k0, r0, m: jnp.concatenate([ld(ref, (*idx, k0 + c), r0, m) for c in range(2)], axis=1)
        xsw_v = xsw_l[i % 2]
        lhs = ((xsw_v, (0,), 0, 0), (xsw_v, (1,), 0, 0), (xpw_l[i % 2], (i // 2,), 0, 0), (xpw_l[i % 2], (i // 2,), 2, HB),
               (xsw_v, (2,), 0, 0), (xsw_v, (3,), 0, 0), (xsw_v, (4,), 0, 0))
        rhs = ((tw_v, (0,), 0), (wgw_v, (), 0), (tw_v, (1,), 0), (tw_v, (2,), 0),
               (wuw_v, (), 2), (tw_v, (3,), 0), (tw_v, (4,), 0))

        def prod(q, k, c0, n):
            def fn():
                ref, idx, k0, r0 = lhs[k]
                m = lax.dot_general(two(ref, idx, k0, r0, HB), two(*rhs[k], c0, n), NT, preferred_element_type=F32)
                if k == 0:
                    val["g1"], val["u2"] = m, m
                elif k == 1:
                    val["g2"], val["u2"] = m, val["u2"] - m
                elif k == 2:
                    val["u1"], val["u2"] = m, val["u2"] + m
                elif k == 3:
                    val["g1"] = val["g1"] + m
                    gu_v[q % 2, 2, :, 0:n] = val.pop("g2") + m
                elif k == 4:
                    val["g1"] = val["g1"] - m
                    gu_v[q % 2, 1, :, 0:n] = val.pop("u1") + m
                elif k == 5:
                    gu_v[q % 2, 3, :, 0:n] = val.pop("u2") + m
                else:
                    gu_v[q % 2, 0, :, 0:n] = val.pop("g1") + m
            return fn

        def act(q, h, c, n):
            def fn():
                w = min(128, n - 128 * c)
                cs = pl.ds(128 * c, w)
                a = (_gelu(gu_v[q % 2, 2 * h, :, cs]) * gu_v[q % 2, 2 * h + 1, :, cs]).astype(BF16)
                a_l[q % 2][c, pl.ds(HB * h, HB), 0:w] = a
            return fn

        def down(q, c0, n):
            def fn():
                if n == FC:
                    a = jnp.concatenate([ld(aw_l[q % 2], (c,), 0, TB) for c in range(FC // 128)], axis=1)
                else:
                    a = a_l[q % 2][0, :, 0:n]
                d = jnp.dot(a, lanes(wdw_v, (), NC, c0, n), preferred_element_type=F32)
                if q == 0:
                    acc_v[i % 2] = d
                else:
                    acc_v[i % 2] += d
            return fn

        items, t, marks = [], t0, []
        pend = None
        for q, (c0, c1) in enumerate(chunks):
            n = c1 - c0
            nt = (n + 127) // 128
            for k in range(7):
                items.append((t, prod(q, k, c0, n)))
                if k == 0:
                    marks.append(t)
                t += nt * T
            tq = t
            parts = [act(q, h, c, n) for c in range(nt) for h in range(2)]
            if pend is not None:
                items.append((t, pend))
                t += 8 * T
            items += [(tq + T + 4 * T * j, f) for j, f in enumerate(parts)]
            pend = down(q, c0, n)
        return items, t, pend, marks

    def gate(i, r0, nr):
        def fn():
            z = None
            for c in range(NC):
                t = (xp_l[i % 2][i // 2, c, pl.ds(r0, nr), :].astype(F32) * st["gw"][c]).astype(BF16).astype(F32)
                z = t if z is None else z + t
            z = jnp.sum(z, axis=-1, keepdims=True).astype(BF16).astype(F32)
            g_v[i % 2, pl.ds(r0, nr), :] = jnp.broadcast_to(jax.nn.sigmoid(z), (nr, 128))
        return fn

    def gates(i):
        return [gate(i, r0, GR) for r0 in range(0, TB, GR)]

    def cproj(i, n):
        def fn():
            y_v[n] = lax.dot_general(lanes(hw_l[i % 2], (), 2 * NC, 0, TB),
                                     lanes(cww_v, (), 2 * NC, 128 * n, 128), NT, preferred_element_type=F32)
        return fn

    def mix(i, n, r0, nr):
        def fn():
            xf = ld(xpw_l[i % 2], (i // 2, n), r0, nr).astype(F32)
            g = g_v[i % 2, pl.ds(r0, nr), :]
            a = y_v[n, pl.ds(r0, nr), :] + (xf * st["dsk"][n]).astype(BF16).astype(F32)
            res = g * a + (1.0 - g) * acc_v[i % 2, pl.ds(r0, nr), cols[n]]
            for j in range(r0 // NS, (r0 + nr) // NS):
                st_v[i, n, pl.ds(j, NS, stride=TJP), :] = res[NS * j - r0:NS * j - r0 + NS, :]
            if r0 + nr == TB and i >= NB - 1:
                o_copy(i, n).start()
        return fn

    def mixes(i, n):
        return [mix(i, n, r0, MR) for r0 in range(0, TB, MR)]

    def discretise():
        wait(vec_copies)
        lre = lre_v[...].astype(F32).reshape(1, P)
        lim = lim_v[...].astype(F32).reshape(1, P)
        dt = jnp.exp(ldt_v[...].astype(F32).reshape(1, P)).astype(BF16).astype(F32)
        mag = jnp.exp(dt * lre)
        lr1 = mag * jnp.cos(dt * lim)
        li1 = mag * jnp.sin(dt * lim)
        big = jnp.maximum(jnp.abs(lre), jnp.abs(lim))
        ur, ui = lre / big, lim / big
        den = (ur * ur + ui * ui) * big
        nr = lr1 - 1.0
        st["kr"] = (nr * ur + li1 * ui) / den
        st["ki"] = (li1 * ur - nr * ui) / den
        lr = jnp.broadcast_to(lr1, (NS, P))
        li = jnp.broadcast_to(li1, (NS, P))
        tiles = lambda v: [v[:, 128 * c:128 * (c + 1)] for c in range(NC)]
        st["lr"], st["li"] = tiles(lr), tiles(li)
        pr, pi = lr1, li1
        for _ in range(8):
            pr, pi = _cmul(pr, pi, pr, pi)
        st["pr"], st["pi"] = tiles(jnp.broadcast_to(pr, (NS, P))), tiles(jnp.broadcast_to(pi, (NS, P)))
        z = jnp.zeros((NS, 128), F32)
        st["er"], st["ei"] = [z] * NC, [z] * NC
        st["gw"] = tiles(gw_v[...].astype(F32).reshape(1, D))
        st["dsk"] = tiles(dsk_v[...].astype(F32).reshape(1, D))

    def cprep(c, h):
        def fn():
            cr = ld(cin_v, (c,), 128 * h, 128).astype(F32)
            ci = ld(cin_v, (c,), D + 128 * h, 128).astype(F32)
            kr, ki = st["kr"][:, 128 * c:128 * (c + 1)], st["ki"][:, 128 * c:128 * (c + 1)]
            wr, wi = _cmul(cr, ci, kr, ki)
            stb(cw_v, (c,), 128 * h, (2.0 * wr).astype(BF16))
            stb(cw_v, (NC + c,), 128 * h, (-2.0 * wi).astype(BF16))
        return fn

    def carry():
        sub = lax.broadcasted_iota(jnp.int32, (NS, 128), 0)
        for c in range(NC):
            ar, ai = st["pr"][c], st["pi"][c]
            er, ei = st["er"][c], st["ei"][c]
            for k in (1, 2, 4):
                tr, ti = _cmul(ar, ai, pltpu.roll(er, k, 0), pltpu.roll(ei, k, 0))
                er, ei = er + jnp.where(sub >= k, tr, 0.0), ei + jnp.where(sub >= k, ti, 0.0)
                ar, ai = _cmul(ar, ai, ar, ai)
            st["er"][c] = jnp.where(sub >= 1, pltpu.roll(er, 1, 0), 0.0)
            st["ei"][c] = jnp.where(sub >= 1, pltpu.roll(ei, 1, 0), 0.0)

    x_copy(0).wait()
    start(cb[1])
    for f in perm_as(0) + perm_bs(0):
        f()
    wait_b(0)
    start(cb[2] + [x_copy(1)])
    starts = {1: [x_copy(4, 4)], 2: c_wg, 3: c_wu, WSTAGE: c_wd + cc_re + cc_im}
    waits = {1: [x_copy(2, 2)], 3: [x_copy(4, 4)], WSTAGE: [whole(wg_v, wsem.at[4]), whole(wu_v, wsem.at[5])]}
    wp = [wprep(c, r0, min(WR, F - r0)) for r0 in range(0, F, WR) for c in range(2)]
    T = 16 * TB // 64

    for i in range(NB):
        main = [(4 * T, bu_mm(i, n)) for n in range(2 * NC)]
        if i == 0:
            main[6:6] = [(0, lambda: (wait_b(3), x_copy(1).wait()))]
            main[4:4] = [(0, lambda: (wait_b(2), x_copy(2, 2).start()))]
            main[2:2] = [(0, lambda: (wait_b(1), start(cb[3])))]
        main, t1 = _seq(0, main)
        side = []
        wait(waits.get(i, []))
        start(starts.get(i, []))
        if i == 1:
            discretise()
        if i == 0:
            side += _spread(t1 * 0.75 + 1, t1 * 0.87, perm_as(1)) + _spread(t1 * 0.87, t1, perm_bs(1))
        elif i + 1 < NB:
            side += _spread(0, t1 * 0.5, perm_as(i + 1))
            side += _spread(t1 * 0.5, t1, perm_bs(i + 1))
        if i >= 1:
            side += _spread(0, t1, scans(i - 1, False))
        if i == XSTAGE:
            side += _spread(0, t1, xsums(0))
        side += _spread(0, t1, wp[len(wp) * (i - WSTAGE) // (NB - WSTAGE):len(wp) * (i + 1 - WSTAGE) // (NB - WSTAGE)] if i >= WSTAGE else [])
        _run(main, side)

    chunks = [(c0, min(c0 + FC, F)) for c0 in range(0, F, FC)]
    pend_down = None

    def wait_wd_c():
        wait([whole(wd_v, wsem.at[6]), whole(c_v.at[:, pl.ds(0, D)], wsem.at[2]),
              whole(c_v.at[:, pl.ds(D, D)], wsem.at[3])])
    for i in range(NB + 1):
        main, side, t1 = [], [], 0
        if i < NB:
            first, t1, last, marks = ffn_items(i, 0)
            main += first
        if i >= 1 and i < NB:
            tp, tc = marks[1], marks[CPQ]
            sh = lambda t: t + (4 * T if t >= tp else 0) + (8 * T * NC if t >= tc else 0)
            main = [(sh(t), f) for t, f in main]
            main.append((tp, pend_down))
            main += [(tc + 4 * T + 8 * T * n, cproj(i - 1, n)) for n in range(NC)]
            t1 = sh(t1)
            tm = tc + 4 * T + 8 * T * NC
            td = min(sh(t) for t in marks if sh(t) > tm + MIXT * T)
            side += _spread(tm, tm + MIXT * T, [f for n in range(NC) for f in mixes(i - 1, n)])
            side += [(td + 0.5, lambda i=i: start([o_copy(i - 1, c) for c in range(NC)]))]
            side += _spread(20 * T, tm, gates(i))
            if i + 1 < NB:
                side += _spread(tm + MIXT * T, t1 - 30 * T, xsums(i + 1))
            side += _spread(0, t1 - 8 * T, scans(i, True))
        elif i == NB:
            main.append((0, pend_down))
            main += [(4 * T + 8 * T * n, cproj(i - 1, n)) for n in range(NC)]
            side += [(4 * T + 8 * T * (n + 1) - 1, f) for n in range(NC) for f in mixes(i - 1, n)]
        else:
            side += _spread(70 * T, t1, gates(0))
            side += _spread(0, 30 * T, xsums(1))
            side += _spread(0, 30 * T, scans(NB - 1, False))
            side += [(30 * T, carry), (marks[1] + 0.5, wait_wd_c)]
            side += _spread(30 * T, 70 * T, [cprep(c, h) for c in range(NC) for h in range(D // 128)])
            side += _spread(40 * T, t1 - 8 * T, scans(i, True))
        if i < NB:
            pend_down = last
        _run(main, side)
    for i in range(NB):
        pltpu.make_async_copy(st5_v.at[i, :, :, pl.ds(0, TJ), :], st5_v.at[i, :, :, pl.ds(0, TJ), :], osem.at[i]).wait()


@jax.jit
def pallas_gated_mix__ssm_conv_s5__geglu_ffn__prompt_kernel(
    A_x, A_Lambda_re, A_Lambda_im, A_B_re, A_B_im, A_C_re, A_C_im, A_log_dt, A_Dskip,
    B_x, B_w_gate, B_w_up, B_w_down, gate_w,
):
    del B_x
    x4 = A_x.reshape(NS, NB, TJ, D)
    hbm = pl.BlockSpec(memory_space=pltpu.HBM)
    out = pl.pallas_call(
        _kernel,
        out_shape=jax.ShapeDtypeStruct((NS, NB, TJ, D), F32),
        in_specs=[hbm] * 13,
        out_specs=hbm,
        scratch_shapes=[
            *[pltpu.VMEM((P,), BF16)] * 5,
            pltpu.VMEM((NS, NB, TJ, D), BF16),
            pltpu.VMEM((NC, NS * TJP, 128), F32),
            *[pltpu.VMEM((NB // 2, NC, TB, 128), BF16)] * 2,
            pltpu.VMEM((NC, 2 * P, 128), BF16),
            pltpu.VMEM((NC, 2 * D, 128), BF16),
            pltpu.VMEM((2 * NC, D, 128), BF16),
            pltpu.VMEM((NC, F, 128), BF16),
            pltpu.VMEM((NC, F, 128), BF16),
            pltpu.VMEM((NC, F, 128), BF16),
            pltpu.VMEM((NB, 2 * NC, TB, 128), F32),
            *[pltpu.VMEM((2 * NC, TB, 128), BF16)] * 2,
            pltpu.VMEM((2, TB, D), F32),
            pltpu.VMEM((2, TB, 128), F32),
            pltpu.VMEM((NC, TB, 128), F32),
            pltpu.VMEM((NB, NC, NS * TJP, 128), F32),
            *[pltpu.VMEM((5, 2, TB // 2, 128), BF16)] * 2,
            pltpu.VMEM((5, 2, F, 128), BF16),
            pltpu.VMEM((2, 4, TB // 2, FC), F32),
            *[pltpu.VMEM((FC // 128, TB, 128), BF16)] * 2,
            pltpu.SemaphoreType.DMA((NB,)),
            pltpu.SemaphoreType.DMA((NB,)),
            pltpu.SemaphoreType.DMA((7,)),
            pltpu.SemaphoreType.DMA((5,)),
            pltpu.SemaphoreType.DMA((4,)),
        ],
        compiler_params=pltpu.CompilerParams(vmem_limit_bytes=64 * 1024 * 1024),
    )(x4, A_Lambda_re, A_Lambda_im, A_B_re, A_B_im, A_C_re, A_C_im, A_log_dt, A_Dskip,
      B_w_gate.T, B_w_up.T, B_w_down, gate_w)
    return out.reshape(1, L, D)
```

```python
import jax
import jax.numpy as jnp
from jax import lax
import jax.experimental.pallas as pl
import jax.experimental.pallas.tpu as pltpu

L, D, P, F = 2048, 512, 512, 1376
NS = 8
SEG = L // NS
TJ = 32
NB = SEG // TJ
TB = NS * TJ
TJP = TJ + 8
NC = D // 128
FC = 256
PR = 32
WR = 32
WSTAGE = 5
CPQ = 2
MIXT = 40
XSTAGE = 2
GR = 32
MR = 64
F32 = jnp.float32
BF16 = jnp.bfloat16
NT = (((1,), (1,)), ((), ()))


def _cmul(ar, ai, br, bi):
    return ar * br - ai * bi, ar * bi + ai * br


def _gelu(g):
    inner = 0.7978845608028654 * (g + 0.044715 * (g * g * g))
    return 0.5 * g * (1.0 + jnp.tanh(inner))


def _run(*timed):
    items = [it for lst in timed for it in lst]
    for n in sorted(range(len(items)), key=lambda k: (items[k][0], k)):
        items[n][1]()


def _seq(t0, pieces):
    out = []
    for dur, fn in pieces:
        out.append((t0, fn))
        t0 += dur
    return out, t0


def _spread(t0, t1, fns):
    fns = list(fns)
    return [(t0 + (t1 - t0) * (n + 0.25) / len(fns), fn) for n, fn in enumerate(fns)]


def _kernel(x_hbm, lre_hbm, lim_hbm, bre_hbm, bim_hbm, cre_hbm, cim_hbm, ldt_hbm, dsk_hbm,
            wg_hbm, wu_hbm, wd_hbm, gw_hbm, out_hbm,
            lre_v, lim_v, ldt_v, dsk_v, gw_v,
            x_v, xf_v, xp0_v, xp1_v, b_v, c_v, cw_v, wg_v, wu_v, wd_v, bu_v, h0_v, h1_v, acc_v, g_v, y_v, st_v, xs0_v, xs1_v, t_v, gu_v, a0_v, a1_v,
            xsem, osem, wsem, vsem, bsem):
    cols = [pl.ds(128 * c, 128) for c in range(NC)]

    st5_v = st_v.reshape(NB, NC, NS, TJP, 128)

    def x_copy(i, n=1):
        return pltpu.make_async_copy(x_hbm.at[:, pl.ds(i, n)], x_v.at[:, pl.ds(i, n)], xsem.at[i])

    def whole(buf, sem):
        return pltpu.make_async_copy(buf, buf, sem)

    def o_copy(i, c):
        return pltpu.make_async_copy(st5_v.at[i, c, :, pl.ds(0, TJ), :],
                                     out_hbm.at[:, i, :, cols[c]], osem.at[i])

    def w_copies(k, src, dst, r0, n):
        return [pltpu.make_async_copy(src.at[:, cols[c]], dst.at[c, pl.ds(r0, n)], wsem.at[k])
                for c in range(NC)]

    QB = 2 * P // 4
    cb = [[pltpu.make_async_copy((bre_hbm, bim_hbm)[q // 2].at[pl.ds(QB * (q % 2), QB), cols[c]],
                                 b_v.at[c, pl.ds(QB * q, QB)], bsem.at[q]) for c in range(NC)]
          for q in range(4)]
    wait_b = lambda q: whole(b_v.at[:, pl.ds(QB * q, QB)], bsem.at[q]).wait()
    cc_re = w_copies(0, cre_hbm, c_v, 0, D)
    cc_im = w_copies(1, cim_hbm, c_v, D, D)
    c_wg = w_copies(2, wg_hbm, wg_v, 0, F)
    c_wu = w_copies(3, wu_hbm, wu_v, 0, F)
    c_wd = w_copies(4, wd_hbm, wd_v, 0, F)
    vec_copies = [pltpu.make_async_copy(s, d, vsem.at[k]) for k, (s, d) in enumerate(
        ((lre_hbm, lre_v), (lim_hbm, lim_v), (ldt_hbm, ldt_v), (dsk_hbm, dsk_v), (gw_hbm, gw_v)))]

    def start(cs):
        for c in cs:
            c.start()

    def wait(cs):
        for c in cs:
            c.wait()

    x_copy(0).start()
    start(cb[0])
    start(vec_copies)
    U32 = jnp.uint32
    bw_v, cin_v = b_v.bitcast(U32), c_v.bitcast(U32)
    cww_v = cw_v.bitcast(U32)
    xp_l, h_l, a_l = (xp0_v, xp1_v), (h0_v, h1_v), (a0_v, a1_v)
    xpw_l, hw_l, aw_l = ([r.bitcast(U32) for r in l] for l in (xp_l, h_l, a_l))
    xs_l = (xs0_v, xs1_v)
    xsw_l, tw_v = [r.bitcast(U32) for r in xs_l], t_v.bitcast(U32)
    wgw_v, wuw_v, wdw_v = wg_v.bitcast(U32), wu_v.bitcast(U32), wd_v.bitcast(U32)

    def ld(ref, idx, r0, n):
        return pltpu.bitcast(ref[(*idx, pl.ds(r0 // 2, n // 2), slice(None))], BF16)

    def stb(ref, idx, r0, val):
        ref[(*idx, pl.ds(r0, val.shape[0]), slice(None))] = val

    def lanes(ref, idx, nc, r0, n):
        return jnp.concatenate([ld(ref, (*idx, c), r0, n) for c in range(nc)], axis=1)

    def perm_a(i, c, s):
        def fn():
            xf_v[c, pl.ds(TJP * s, TJ), :] = x_v[s, i, :, cols[c]].astype(F32)
        return fn

    def perm_as(i):
        return [perm_a(i, c, s) for c in (0, 2, 1, 3) for s in range(NS)]

    HB = TB // 2

    def perm_b(i, c, r0):
        def fn():
            rows = lambda cc, r: jnp.concatenate(
                [xf_v[cc, pl.ds(j, NS, stride=TJP), :] for j in range(r // NS, (r + PR) // NS)], axis=0)
            a11, a21, a12, a22 = rows(c, r0), rows(c, HB + r0), rows(c + 2, r0), rows(c + 2, HB + r0)
            stb(xp_l[i % 2], (i // 2, c), r0, a11.astype(BF16))
            stb(xp_l[i % 2], (i // 2, c), HB + r0, a21.astype(BF16))
            stb(xp_l[i % 2], (i // 2, c + 2), r0, a12.astype(BF16))
            stb(xp_l[i % 2], (i // 2, c + 2), HB + r0, a22.astype(BF16))
        return fn

    def xsum(i, c, r0):
        def fn():
            q = lambda cc, r: ld(xpw_l[i % 2], (i // 2, cc), r, PR).astype(F32)
            a11, a21, a12, a22 = q(c, r0), q(c, HB + r0), q(c + 2, r0), q(c + 2, HB + r0)
            for k, v in enumerate((a11 + a22, a21 + a22, a11 + a12, a21 - a11, a12 - a22)):
                stb(xs_l[i % 2], (k, c), r0, v.astype(BF16))
        return fn

    def xsums(i):
        return [xsum(i, c, r0) for c in range(2) for r0 in range(0, HB, PR)]

    def perm_bs(i):
        return [perm_b(i, c, r0) for c in range(2) for r0 in range(0, HB, PR)]

    def wprep(c, r0, n):
        def fn():
            b11 = ld(wgw_v, (c,), r0, n).astype(F32)
            b21 = ld(wgw_v, (c + 2,), r0, n).astype(F32)
            b12 = ld(wuw_v, (c,), r0, n).astype(F32)
            b22 = ld(wuw_v, (c + 2,), r0, n).astype(F32)
            for k, v in enumerate((b11 + b22, b12 - b22, b21 - b11, b11 + b12, b21 + b22)):
                stb(t_v, (k, c), r0, v.astype(BF16))
        return fn

    def bu_mm(i, n):
        def fn():
            w = lanes(bw_v, (), NC, 128 * n, 128)
            bu_v[i, n] = lax.dot_general(lanes(xpw_l[i % 2], (i // 2,), NC, 0, TB), w, NT, preferred_element_type=F32)
        return fn

    st = {}

    def scan(i, j, store):
        def fn():
            er, ei = st["er"], st["ei"]
            lr, li = st["lr"], st["li"]
            for c in range(NC):
                hs = []
                for jj in (j, j + 1):
                    br = bu_v[i, c, pl.ds(NS * jj, NS), :]
                    bi = bu_v[i, NC + c, pl.ds(NS * jj, NS), :]
                    er[c], ei[c] = lr[c] * er[c] - li[c] * ei[c] + br, lr[c] * ei[c] + li[c] * er[c] + bi
                    hs.append((er[c], ei[c]))
                if store:
                    stb(h_l[i % 2], (c,), NS * j, jnp.concatenate([hs[0][0], hs[1][0]], axis=0).astype(BF16))
                    stb(h_l[i % 2], (NC + c,), NS * j, jnp.concatenate([hs[0][1], hs[1][1]], axis=0).astype(BF16))
        return fn

    def scans(i, store):
        return [scan(i, j, store) for j in range(0, TJ, 2)]

    def ffn_items(i, t0):
        val = {}
        two = lambda ref, idx, k0, r0, m: jnp.concatenate([ld(ref, (*idx, k0 + c), r0, m) for c in range(2)], axis=1)
        xsw_v = xsw_l[i % 2]
        lhs = ((xsw_v, (0,), 0, 0), (xsw_v, (1,), 0, 0), (xpw_l[i % 2], (i // 2,), 0, 0), (xpw_l[i % 2], (i // 2,), 2, HB),
               (xsw_v, (2,), 0, 0), (xsw_v, (3,), 0, 0), (xsw_v, (4,), 0, 0))
        rhs = ((tw_v, (0,), 0), (wgw_v, (), 0), (tw_v, (1,), 0), (tw_v, (2,), 0),
               (wuw_v, (), 2), (tw_v, (3,), 0), (tw_v, (4,), 0))

        def prod(q, k, c0, n):
            def fn():
                ref, idx, k0, r0 = lhs[k]
                m = lax.dot_general(two(ref, idx, k0, r0, HB), two(*rhs[k], c0, n), NT, preferred_element_type=F32)
                if k == 0:
                    val["g1"], val["u2"] = m, m
                elif k == 1:
                    val["g2"], val["u2"] = m, val["u2"] - m
                elif k == 2:
                    val["u1"], val["u2"] = m, val["u2"] + m
                elif k == 3:
                    val["g1"] = val["g1"] + m
                    gu_v[q % 2, 2, :, 0:n] = val.pop("g2") + m
                elif k == 4:
                    val["g1"] = val["g1"] - m
                    gu_v[q % 2, 1, :, 0:n] = val.pop("u1") + m
                elif k == 5:
                    gu_v[q % 2, 3, :, 0:n] = val.pop("u2") + m
                else:
                    gu_v[q % 2, 0, :, 0:n] = val.pop("g1") + m
            return fn

        def act(q, h, c, n):
            def fn():
                w = min(128, n - 128 * c)
                cs = pl.ds(128 * c, w)
                a = (_gelu(gu_v[q % 2, 2 * h, :, cs]) * gu_v[q % 2, 2 * h + 1, :, cs]).astype(BF16)
                a_l[q % 2][c, pl.ds(HB * h, HB), 0:w] = a
            return fn

        def down(q, c0, n):
            def fn():
                if n == FC:
                    a = jnp.concatenate([ld(aw_l[q % 2], (c,), 0, TB) for c in range(FC // 128)], axis=1)
                else:
                    a = a_l[q % 2][0, :, 0:n]
                d = jnp.dot(a, lanes(wdw_v, (), NC, c0, n), preferred_element_type=F32)
                if q == 0:
                    acc_v[i % 2] = d
                else:
                    acc_v[i % 2] += d
            return fn

        items, t, marks = [], t0, []
        pend = None
        for q, (c0, c1) in enumerate(chunks):
            n = c1 - c0
            nt = (n + 127) // 128
            for k in range(7):
                items.append((t, prod(q, k, c0, n)))
                if k == 0:
                    marks.append(t)
                t += nt * T
            tq = t
            parts = [act(q, h, c, n) for c in range(nt) for h in range(2)]
            if pend is not None:
                items.append((t, pend))
                t += 8 * T
            items += [(tq + T + 4 * T * j, f) for j, f in enumerate(parts)]
            pend = down(q, c0, n)
        return items, t, pend, marks

    def gate(i, r0, nr):
        def fn():
            z = None
            for c in range(NC):
                t = (xp_l[i % 2][i // 2, c, pl.ds(r0, nr), :].astype(F32) * st["gw"][c]).astype(BF16).astype(F32)
                z = t if z is None else z + t
            z = jnp.sum(z, axis=-1, keepdims=True).astype(BF16).astype(F32)
            g_v[i % 2, pl.ds(r0, nr), :] = jnp.broadcast_to(jax.nn.sigmoid(z), (nr, 128))
        return fn

    def gates(i):
        return [gate(i, r0, GR) for r0 in range(0, TB, GR)]

    def cproj(i, n):
        def fn():
            y_v[n] = lax.dot_general(lanes(hw_l[i % 2], (), 2 * NC, 0, TB),
                                     lanes(cww_v, (), 2 * NC, 128 * n, 128), NT, preferred_element_type=F32)
        return fn

    def mix(i, n, r0, nr):
        def fn():
            xf = ld(xpw_l[i % 2], (i // 2, n), r0, nr).astype(F32)
            g = g_v[i % 2, pl.ds(r0, nr), :]
            a = y_v[n, pl.ds(r0, nr), :] + (xf * st["dsk"][n]).astype(BF16).astype(F32)
            res = g * a + (1.0 - g) * acc_v[i % 2, pl.ds(r0, nr), cols[n]]
            for j in range(r0 // NS, (r0 + nr) // NS):
                st_v[i, n, pl.ds(j, NS, stride=TJP), :] = res[NS * j - r0:NS * j - r0 + NS, :]
            if r0 + nr == TB and i >= NB - 1:
                o_copy(i, n).start()
        return fn

    def mixes(i, n):
        return [mix(i, n, r0, MR) for r0 in range(0, TB, MR)]

    def discretise():
        wait(vec_copies)
        lre = lre_v[...].astype(F32).reshape(1, P)
        lim = lim_v[...].astype(F32).reshape(1, P)
        dt = jnp.exp(ldt_v[...].astype(F32).reshape(1, P)).astype(BF16).astype(F32)
        mag = jnp.exp(dt * lre)
        lr1 = mag * jnp.cos(dt * lim)
        li1 = mag * jnp.sin(dt * lim)
        big = jnp.maximum(jnp.abs(lre), jnp.abs(lim))
        ur, ui = lre / big, lim / big
        den = (ur * ur + ui * ui) * big
        nr = lr1 - 1.0
        st["kr"] = (nr * ur + li1 * ui) / den
        st["ki"] = (li1 * ur - nr * ui) / den
        lr = jnp.broadcast_to(lr1, (NS, P))
        li = jnp.broadcast_to(li1, (NS, P))
        tiles = lambda v: [v[:, 128 * c:128 * (c + 1)] for c in range(NC)]
        st["lr"], st["li"] = tiles(lr), tiles(li)
        pr, pi = lr1, li1
        for _ in range(8):
            pr, pi = _cmul(pr, pi, pr, pi)
        st["pr"], st["pi"] = tiles(jnp.broadcast_to(pr, (NS, P))), tiles(jnp.broadcast_to(pi, (NS, P)))
        z = jnp.zeros((NS, 128), F32)
        st["er"], st["ei"] = [z] * NC, [z] * NC
        st["gw"] = tiles(gw_v[...].astype(F32).reshape(1, D))
        st["dsk"] = tiles(dsk_v[...].astype(F32).reshape(1, D))

    def cprep(c, h):
        def fn():
            cr = ld(cin_v, (c,), 128 * h, 128).astype(F32)
            ci = ld(cin_v, (c,), D + 128 * h, 128).astype(F32)
            kr, ki = st["kr"][:, 128 * c:128 * (c + 1)], st["ki"][:, 128 * c:128 * (c + 1)]
            wr, wi = _cmul(cr, ci, kr, ki)
            stb(cw_v, (c,), 128 * h, (2.0 * wr).astype(BF16))
            stb(cw_v, (NC + c,), 128 * h, (-2.0 * wi).astype(BF16))
        return fn

    def carry():
        sub = lax.broadcasted_iota(jnp.int32, (NS, 128), 0)
        for c in range(NC):
            ar, ai = st["pr"][c], st["pi"][c]
            er, ei = st["er"][c], st["ei"][c]
            for k in (1, 2, 4):
                tr, ti = _cmul(ar, ai, pltpu.roll(er, k, 0), pltpu.roll(ei, k, 0))
                er, ei = er + jnp.where(sub >= k, tr, 0.0), ei + jnp.where(sub >= k, ti, 0.0)
                ar, ai = _cmul(ar, ai, ar, ai)
            st["er"][c] = jnp.where(sub >= 1, pltpu.roll(er, 1, 0), 0.0)
            st["ei"][c] = jnp.where(sub >= 1, pltpu.roll(ei, 1, 0), 0.0)

    x_copy(0).wait()
    start(cb[1])
    for f in perm_as(0) + perm_bs(0):
        f()
    wait_b(0)
    start(cb[2] + [x_copy(1)])
    starts = {1: [x_copy(4, 4)], 2: c_wg, 3: c_wu, WSTAGE: c_wd + cc_re + cc_im}
    waits = {1: [x_copy(2, 2)], 3: [x_copy(4, 4)], WSTAGE: [whole(wg_v, wsem.at[2]), whole(wu_v, wsem.at[3])]}
    wp = [wprep(c, r0, min(WR, F - r0)) for r0 in range(0, F, WR) for c in range(2)]
    T = 16 * TB // 64

    for i in range(NB):
        main = [(4 * T, bu_mm(i, n)) for n in range(2 * NC)]
        if i == 0:
            main[6:6] = [(0, lambda: (wait_b(3), x_copy(1).wait()))]
            main[4:4] = [(0, lambda: (wait_b(2), x_copy(2, 2).start()))]
            main[2:2] = [(0, lambda: (wait_b(1), start(cb[3])))]
        main, t1 = _seq(0, main)
        side = []
        wait(waits.get(i, []))
        start(starts.get(i, []))
        if i == 1:
            discretise()
        if i == 0:
            side += _spread(t1 * 0.75 + 1, t1 * 0.87, perm_as(1)) + _spread(t1 * 0.87, t1, perm_bs(1))
        elif i + 1 < NB:
            side += _spread(0, t1 * 0.5, perm_as(i + 1))
            side += _spread(t1 * 0.5, t1, perm_bs(i + 1))
        if i >= 1:
            side += _spread(0, t1, scans(i - 1, False))
        if i == XSTAGE:
            side += _spread(0, t1, xsums(0))
        side += _spread(0, t1, wp[len(wp) * (i - WSTAGE) // (NB - WSTAGE):len(wp) * (i + 1 - WSTAGE) // (NB - WSTAGE)] if i >= WSTAGE else [])
        _run(main, side)

    chunks = [(c0, min(c0 + FC, F)) for c0 in range(0, F, FC)]
    pend_down = None

    def wait_wd_c():
        wait([whole(wd_v, wsem.at[4]), whole(c_v.at[:, pl.ds(0, D)], wsem.at[0]),
              whole(c_v.at[:, pl.ds(D, D)], wsem.at[1])])
    for i in range(NB + 1):
        main, side, t1 = [], [], 0
        if i < NB:
            first, t1, last, marks = ffn_items(i, 0)
            main += first
        if i >= 1 and i < NB:
            tp, tc = marks[1], marks[CPQ]
            sh = lambda t: t + (4 * T if t >= tp else 0) + (8 * T * NC if t >= tc else 0)
            main = [(sh(t), f) for t, f in main]
            main.append((tp, pend_down))
            main += [(tc + 4 * T + 8 * T * n, cproj(i - 1, n)) for n in range(NC)]
            t1 = sh(t1)
            tm = tc + 4 * T + 8 * T * NC
            td = min(sh(t) for t in marks if sh(t) > tm + MIXT * T)
            side += _spread(tm, tm + MIXT * T, [f for n in range(NC) for f in mixes(i - 1, n)])
            side += [(td + 0.5, lambda i=i: start([o_copy(i - 1, c) for c in range(NC)]))]
            side += _spread(20 * T, tm, gates(i))
            if i + 1 < NB:
                side += _spread(tm + MIXT * T, t1 - 30 * T, xsums(i + 1))
            side += _spread(0, t1 - 8 * T, scans(i, True))
        elif i == NB:
            main.append((0, pend_down))
            main += [(4 * T + 8 * T * n, cproj(i - 1, n)) for n in range(NC)]
            side += [(4 * T + 8 * T * (n + 1) - 1, f) for n in range(NC) for f in mixes(i - 1, n)]
        else:
            side += _spread(70 * T, t1, gates(0))
            side += _spread(0, 30 * T, xsums(1))
            side += _spread(0, 30 * T, scans(NB - 1, False))
            side += [(30 * T, carry), (marks[1] + 0.5, wait_wd_c)]
            side += _spread(30 * T, 70 * T, [cprep(c, h) for c in range(NC) for h in range(D // 128)])
            side += _spread(40 * T, t1 - 8 * T, scans(i, True))
        if i < NB:
            pend_down = last
        _run(main, side)
    for i in range(NB):
        whole(out_hbm.at[:, i], osem.at[i]).wait()


@jax.jit
def pallas_gated_mix__ssm_conv_s5__geglu_ffn__prompt_kernel(
    A_x, A_Lambda_re, A_Lambda_im, A_B_re, A_B_im, A_C_re, A_C_im, A_log_dt, A_Dskip,
    B_x, B_w_gate, B_w_up, B_w_down, gate_w,
):
    del B_x
    x4 = A_x.reshape(NS, NB, TJ, D)
    hbm = pl.BlockSpec(memory_space=pltpu.HBM)
    out = pl.pallas_call(
        _kernel,
        out_shape=jax.ShapeDtypeStruct((NS, NB, TJ, D), F32),
        in_specs=[hbm] * 13,
        out_specs=hbm,
        scratch_shapes=[
            *[pltpu.VMEM((P,), BF16)] * 5,
            pltpu.VMEM((NS, NB, TJ, D), BF16),
            pltpu.VMEM((NC, NS * TJP, 128), F32),
            *[pltpu.VMEM((NB // 2, NC, TB, 128), BF16)] * 2,
            pltpu.VMEM((NC, 2 * P, 128), BF16),
            pltpu.VMEM((NC, 2 * D, 128), BF16),
            pltpu.VMEM((2 * NC, D, 128), BF16),
            pltpu.VMEM((NC, F, 128), BF16),
            pltpu.VMEM((NC, F, 128), BF16),
            pltpu.VMEM((NC, F, 128), BF16),
            pltpu.VMEM((NB, 2 * NC, TB, 128), F32),
            *[pltpu.VMEM((2 * NC, TB, 128), BF16)] * 2,
            pltpu.VMEM((2, TB, D), F32),
            pltpu.VMEM((2, TB, 128), F32),
            pltpu.VMEM((NC, TB, 128), F32),
            pltpu.VMEM((NB, NC, NS * TJP, 128), F32),
            *[pltpu.VMEM((5, 2, TB // 2, 128), BF16)] * 2,
            pltpu.VMEM((5, 2, F, 128), BF16),
            pltpu.VMEM((2, 4, TB // 2, FC), F32),
            *[pltpu.VMEM((FC // 128, TB, 128), BF16)] * 2,
            pltpu.SemaphoreType.DMA((NB,)),
            pltpu.SemaphoreType.DMA((NB,)),
            pltpu.SemaphoreType.DMA((5,)),
            pltpu.SemaphoreType.DMA((5,)),
            pltpu.SemaphoreType.DMA((4,)),
        ],
        compiler_params=pltpu.CompilerParams(vmem_limit_bytes=64 * 1024 * 1024),
    )(x4, A_Lambda_re, A_Lambda_im, A_B_re, A_B_im, A_C_re, A_C_im, A_log_dt, A_Dskip,
      B_w_gate.T, B_w_up.T, B_w_down, gate_w)
    return out.reshape(1, L, D)
```
